```python
import jax
import jax.numpy as jnp

def _softmax(x, axis=-1):
    return jax.nn.softmax(x, axis=axis)
def _gelu(x):
    return jax.nn.gelu(x, approximate=True)
def _silu(x):
    return jax.nn.silu(x)
def _sigmoid(x):
    return jax.nn.sigmoid(x)
def _layernorm(x, axis=-1, eps=1e-5):
    m = jnp.mean(x, axis=axis, keepdims=True)
    v = jnp.var(x, axis=axis, keepdims=True)
    return (x - m) / jnp.sqrt(v + eps)
def _scatter_add(tgt, idx, src, axis=0):
    return tgt.at[idx].add(src)
def _segment_sum(src, seg, n):
    return jax.ops.segment_sum(src, seg, n)
class _Rng:
    def __init__(self, key):
        self._k = key
    def _next(self):
        self._k, sub = jax.random.split(self._k)
        return sub
    def normal(self, shape):
        return jax.random.normal(self._next(), shape, dtype=jnp.bfloat16)
    def randint(self, lo, hi, shape):
        return jax.random.randint(self._next(), shape, lo, hi, dtype=jnp.int32)
    def uniform(self, shape, lo=0.0, hi=1.0):
        return jax.random.uniform(self._next(), shape, jnp.bfloat16, lo, hi)
    def permutation(self, n):
        return jax.random.permutation(self._next(), n)


kernel_name = 'recurrent_scan__sliding_block_cached__mixer_s_mlp__decode'

def setup_inputs():
    _rng = _Rng(jax.random.key(int.from_bytes(__import__("os").urandom(4), "little")))
    _w = (lambda a: (lambda t: t.astype(jnp.bfloat16) if jnp.issubdtype(t.dtype, jnp.floating) else t)(jnp.asarray(a)))
    def _A_setup():
        B, Sq, D = 1, 1, 512
        Hq, Hkv, Sk, Dh = 32, 32, 32768, 128
        assert Hq % Hkv == 0, (Hq, Hkv)
        return {
            "x": _w((lambda *s: _rng.normal(s) * 0.05)(B, Sq, D)),
            "k_cache": _w((lambda *s: _rng.normal(s) * 0.05)(B, Hkv, Sk, Dh)),
            "v_cache": _w((lambda *s: _rng.normal(s) * 0.05)(B, Hkv, Sk, Dh)),
            "wq": _w((lambda *s: _rng.normal(s) * 0.05)(D, Hq * Dh) * (D ** -0.5)),
            "wo": _w((lambda *s: _rng.normal(s) * 0.05)(Hq * Dh, D) * ((Hq * Dh) ** -0.5)),
        }
    _A_in = _A_setup()

    def _B_setup():
        B, S, D, F = 1, 1, 512, 1376
        return {
            "x":  _w((lambda *s: _rng.normal(s) * 0.05)(B, S, D)),
            "w1": _w((lambda *s: _rng.normal(s) * 0.05)(D, D) * (D ** -0.5)),
            "w2": _w((lambda *s: _rng.normal(s) * 0.05)(D, D) * (D ** -0.5)),
            "w3": _w((lambda *s: _rng.normal(s) * 0.05)(D, F) * (D ** -0.5)),
            "w4": _w((lambda *s: _rng.normal(s) * 0.05)(F, D) * (F ** -0.5)),
        }
    _B_in = _B_setup()

    return {
        "A_x": _A_in["x"],
        "A_k_cache": _A_in["k_cache"],
        "A_v_cache": _A_in["v_cache"],
        "A_wq": _A_in["wq"],
        "A_wo": _A_in["wo"],
        "B_x": _B_in["x"],
        "B_w1": _B_in["w1"],
        "B_w2": _B_in["w2"],
        "B_w3": _B_in["w3"],
        "B_w4": _B_in["w4"],
    }

def reference(A_x, A_k_cache, A_v_cache, A_wq, A_wo, B_x, B_w1, B_w2, B_w3, B_w4):
    def _A_ref(x, k_cache, v_cache, wq, wo):
        B, Sq, D = x.shape
        Hq, Dh = 32, 128
        Hkv, Sk = k_cache.shape[1], k_cache.shape[2]
        W = min(4096, max(256, Sk // 4))
        rep = Hq // Hkv
        q = (lambda x, *d: x.transpose(*d))((x @ wq).reshape(B, Sq, Hq, Dh), 0, 2, 1, 3)
        k = jnp.repeat(k_cache[:, :, Sk - W:, :], rep, axis=1)
        v = jnp.repeat(v_cache[:, :, Sk - W:, :], rep, axis=1)
        scores = jnp.einsum("bhqd,bhkd->bhqk", q, k) * (Dh ** -0.5)
        p = _softmax(scores, axis=-1)
        o = jnp.einsum("bhqk,bhkd->bhqd", p, v)
        return (lambda x, *d: x.transpose(*d))(o, 0, 2, 1, 3).reshape(B, Sq, Hq * Dh) @ wo

    def _B_ref(x, w1, w2, w3, w4):
        B, S, D = x.shape
        h = _gelu(_layernorm(x, axis=-1) @ w1)
        c = D // 4
        g0 = jnp.pad(h[:, :, 0*c:1*c], ((0, 0), (1, 0), (0, 0)))[:, :S, :]
        g1 = jnp.pad(h[:, :, 1*c:2*c], ((0, 0), (0, 1), (0, 0)))[:, 1:, :]
        g2 = jnp.pad(h[:, :, 2*c:3*c], ((0, 0), (2, 0), (0, 0)))[:, :S, :]
        g3 = jnp.pad(h[:, :, 3*c:   ], ((0, 0), (0, 2), (0, 0)))[:, 2:, :]
        hs = jnp.concatenate([g0, g1, g2, g3], axis=-1) @ w2
        x1 = x + hs
        h2 = _gelu(_layernorm(x1, axis=-1) @ w3) @ w4
        return x1 + h2

    x = A_x
    xn = _layernorm(x, axis=-1)
    s = _A_ref(xn, A_k_cache, A_v_cache, A_wq, A_wo)
    g = _silu(_B_ref(xn, B_w1, B_w2, B_w3, B_w4))
    return x + s * g
```

```python
import functools
import jax
import jax.numpy as jnp
from jax import lax
from jax.experimental import pallas as pl
from jax.experimental.pallas import tpu as pltpu

F32, BF16 = jnp.float32, jnp.bfloat16
NT = (((1,), (1,)), ((), ()))


def _ln(x):
    m = jnp.mean(x, axis=-1, keepdims=True)
    d = x - m
    v = jnp.mean(d * d, axis=-1, keepdims=True)
    return d / jnp.sqrt(v + 1e-5)


def make(G=4, NWO=8, alt=False, window=8):
    def fn(x, k, v, wq, wo, bx, w1, w2, w3, w4):
        _, H, SK, DH = k.shape
        D = x.shape[-1]
        F = w3.shape[1]
        W = min(4096, max(256, SK // 4))
        NG = H // G
        CW = H * DH // NWO

        def kern(x_h, k_h, v_h, wq_h, wo_h, w3_h, w4_h, o_ref,
                 x_v, k_v, v_v, wq_v, wo_v, w3_v, w4_v, q_v, a_v, sems):
            jobs = [(x_h, x_v), (wq_h, wq_v)]
            for g in range(NG):
                jobs.append((k_h.at[0, pl.ds(g * G, G), pl.ds(SK - W, W)], k_v.at[pl.ds(g * G, G)]))
                jobs.append((v_h.at[0, pl.ds(g * G, G), pl.ds(SK - W, W)], v_v.at[pl.ds(g * G, G)]))
            jobs += [(w3_h, w3_v), (w4_h, w4_v)]
            for c in range(NWO):
                jobs.append((wo_h.at[pl.ds(c * CW, CW)], wo_v.at[pl.ds(c * CW, CW)]))
            cps = [pltpu.make_async_copy(s, d, sems.at[i]) for i, (s, d) in enumerate(jobs)]
            n = len(cps)

            def start(i):
                if i < n:
                    cps[i].start(priority=(i % 2 if alt else 0))

            for i in range(window):
                start(i)
            nxt = [0]

            def wait_next():
                i = nxt[0]
                cps[i].wait()
                start(i + window)
                nxt[0] += 1

            wait_next()
            xf = x_v[0].astype(F32)
            xn = _ln(xf).astype(BF16)
            xn2 = _ln(xn.astype(F32)).astype(BF16)
            wait_next()
            q = jnp.dot(xn, wq_v[...], preferred_element_type=F32).astype(BF16)
            for h in range(H):
                q_v[h] = jnp.broadcast_to(q[:, h * DH:(h + 1) * DH], (16, DH))
            scale = DH ** -0.5
            for g in range(NG):
                wait_next()
                wait_next()

                def body(i, _):
                    h = g * G + i
                    s = lax.dot_general(q_v[h], k_v[h], NT, preferred_element_type=F32) * scale
                    m = jnp.max(s, axis=-1, keepdims=True)
                    p = jnp.exp(s - m)
                    l = jnp.sum(p, axis=-1, keepdims=True)
                    o = jnp.dot(p.astype(BF16), v_v[h], preferred_element_type=F32) / l
                    a_v[:, pl.ds(pl.multiple_of(h * DH, DH), DH)] = o.astype(BF16)
                    return 0
                lax.fori_loop(0, G, body, 0)
            wait_next()
            hh = lax.dot_general(xn2, w3_v[...], NT, preferred_element_type=F32)
            hh = jax.nn.gelu(hh.astype(BF16).astype(F32), approximate=True).astype(BF16)
            wait_next()
            h2 = jnp.dot(hh, w4_v[...], preferred_element_type=F32)
            y = xn.astype(F32) + h2
            gate = y * jax.nn.sigmoid(y)
            acc = jnp.zeros((16, D), F32)
            for c in range(NWO):
                wait_next()
                acc = acc + jnp.dot(a_v[:, c * CW:(c + 1) * CW], wo_v[c * CW:(c + 1) * CW, :], preferred_element_type=F32)
            o_ref[0] = (xf + acc[0:1] * gate).astype(o_ref.dtype)

        njobs = 4 + 2 * NG + NWO
        return pl.pallas_call(
            kern,
            in_specs=[pl.BlockSpec(memory_space=pl.ANY)] * 7,
            out_specs=pl.BlockSpec(memory_space=pltpu.VMEM),
            out_shape=jax.ShapeDtypeStruct(x.shape, x.dtype),
            scratch_shapes=[
                pltpu.VMEM(x.shape, BF16), pltpu.VMEM((H, W, DH), BF16), pltpu.VMEM((H, W, DH), BF16),
                pltpu.VMEM(wq.shape, BF16), pltpu.VMEM(wo.shape, BF16), pltpu.VMEM((F, D), BF16), pltpu.VMEM((F, D), BF16),
                pltpu.VMEM((H, 16, DH), BF16), pltpu.VMEM((16, H * DH), BF16),
                pltpu.SemaphoreType.DMA((njobs,))],
            compiler_params=pltpu.CompilerParams(vmem_limit_bytes=100 * 1024 * 1024),
        )(x, k, v, wq, wo, w3.T, w4)
    return fn


_impl = make()


@jax.jit
def pallas_recurrent_scan__sliding_block_cached__mixer_s_mlp__decode_kernel(
    A_x, A_k_cache, A_v_cache, A_wq, A_wo, B_x, B_w1, B_w2, B_w3, B_w4
):
    return _impl(A_x, A_k_cache, A_v_cache, A_wq, A_wo, B_x, B_w1, B_w2, B_w3, B_w4)
```

```python
import jax
import jax.numpy as jnp
from jax import lax
from jax.experimental import pallas as pl
from jax.experimental.pallas import tpu as pltpu

F32, BF16 = jnp.float32, jnp.bfloat16
NT = (((1,), (1,)), ((), ()))


def _ln(x):
    m = jnp.mean(x, axis=-1, keepdims=True)
    d = x - m
    v = jnp.mean(d * d, axis=-1, keepdims=True)
    return d / jnp.sqrt(v + 1e-5)


def make(KG=(16, 16), VG=(8, 8, 4, 4, 4, 2, 2), OG=(16, 8, 4, 3, 1), window=100, alt=False, xfirst=False):
    def fn(x, k, v, wq, wo, bx, w1, w2, w3, w4):
        _, H, SK, DH = k.shape
        D = x.shape[-1]
        F = w3.shape[1]
        W = min(4096, max(256, SK // 4))

        def starts(gs):
            out, s = [], 0
            for g in gs:
                out.append((s, g)); s += g
            assert s == H
            return out

        def kern(x_h, k_h, v_h, wq_h, wo_h, w3_h, w4_h, o_ref,
                 x_v, k_v, v_v, wq_v, wo_v, w3_v, w4_v, a_v, sems):
            jobs = [('wq', 0, wq_h, wq_v), ('x', 0, x_h, x_v)]
            if xfirst: jobs = jobs[::-1]
            kv = [(s, 0, 'k', g) for s, g in starts(KG)] + [(s, 1, 'v', g) for s, g in starts(VG)]
            for s, _, nm, g in sorted(kv):
                src, dst = (k_h, k_v) if nm == 'k' else (v_h, v_v)
                jobs.append((nm, s, src.at[0, pl.ds(s, g), pl.ds(SK - W, W)], dst.at[pl.ds(s, g)]))
            jobs += [('w3', 0, w3_h, w3_v), ('w4', 0, w4_h, w4_v)]
            for s, g in starts(OG):
                jobs.append(('wo', s, wo_h.at[pl.ds(s * DH, g * DH)], wo_v.at[pl.ds(s * DH, g * DH)]))
            cps = [pltpu.make_async_copy(j[2], j[3], sems.at[i]) for i, j in enumerate(jobs)]
            idx = {(j[0], j[1]): i for i, j in enumerate(jobs)}
            n = len(cps)

            def start(i):
                if i < n:
                    cps[i].start(priority=(i % 2 if alt else 0))

            for i in range(window):
                start(i)

            def wait(nm, s=0):
                i = idx[(nm, s)]
                cps[i].wait()
                start(i + window)

            if not xfirst: wait('wq')
            wait('x')
            xf = x_v[0].astype(F32)
            xn = _ln(xf).astype(BF16)
            xn2 = _ln(xn.astype(F32)).astype(BF16)
            xb = jnp.broadcast_to(xn, (16, D))
            if xfirst: wait('wq')
            scale = DH ** -0.5

            def body(h, _):
                col = pl.ds(pl.multiple_of(h * DH, DH), DH)
                q = jnp.dot(xb, wq_v[:, col], preferred_element_type=F32).astype(BF16)
                for s0, _g in starts(KG):
                    pl.when(h == s0)(lambda s0=s0: wait('k', s0))
                for s0, _g in starts(VG):
                    pl.when(h == s0)(lambda s0=s0: wait('v', s0))
                s = lax.dot_general(q, k_v[h], NT, preferred_element_type=F32) * scale
                m = jnp.max(s, axis=-1, keepdims=True)
                p = jnp.exp(s - m)
                l = jnp.sum(p, axis=-1, keepdims=True)
                o = jnp.dot(p.astype(BF16), v_v[h], preferred_element_type=F32) / l
                a_v[h] = o.astype(BF16)
                return 0
            lax.fori_loop(0, H, body, 0)
            wait('w3')
            hh = lax.dot_general(xn2, w3_v[...], NT, preferred_element_type=F32)
            hh = jax.nn.gelu(hh.astype(BF16).astype(F32), approximate=True).astype(BF16)
            wait('w4')
            h2 = jnp.dot(hh, w4_v[...], preferred_element_type=F32)
            y = xn.astype(F32) + h2
            gate = y * jax.nn.sigmoid(y)

            acc = jnp.zeros((16, D), F32)
            for s0, g in starts(OG):
                wait('wo', s0)
                lhs = jnp.concatenate([a_v[s0 + i] for i in range(g)], axis=-1)
                acc = acc + jnp.dot(lhs, wo_v[s0 * DH:(s0 + g) * DH, :], preferred_element_type=F32)
            o_ref[0] = (xf + acc[0:1] * gate).astype(o_ref.dtype)

        njobs = 4 + len(KG) + len(VG) + len(OG)
        return pl.pallas_call(
            kern,
            in_specs=[pl.BlockSpec(memory_space=pl.ANY)] * 7,
            out_specs=pl.BlockSpec(memory_space=pltpu.VMEM),
            out_shape=jax.ShapeDtypeStruct(x.shape, x.dtype),
            scratch_shapes=[
                pltpu.VMEM(x.shape, BF16), pltpu.VMEM((H, W, DH), BF16), pltpu.VMEM((H, W, DH), BF16),
                pltpu.VMEM(wq.shape, BF16), pltpu.VMEM(wo.shape, BF16), pltpu.VMEM((F, D), BF16), pltpu.VMEM((F, D), BF16),
                pltpu.VMEM((H, 16, DH), BF16),
                pltpu.SemaphoreType.DMA((njobs,))],
            compiler_params=pltpu.CompilerParams(vmem_limit_bytes=100 * 1024 * 1024),
        )(x, k, v, wq, wo, w3.T, w4)
    return fn


_impl = make()


@jax.jit
def pallas_recurrent_scan__sliding_block_cached__mixer_s_mlp__decode_kernel(
    A_x, A_k_cache, A_v_cache, A_wq, A_wo, B_x, B_w1, B_w2, B_w3, B_w4
):
    assert A_x.shape[:2] == (1, 1)
    return _impl(A_x, A_k_cache, A_v_cache, A_wq, A_wo, B_x, B_w1, B_w2, B_w3, B_w4)
```
